```python
import os as _os
_os.environ.setdefault("JAX_PLATFORMS", "cpu")
import jax
import jax.numpy as jnp

def _softmax(x, axis=-1):
    return jax.nn.softmax(x, axis=axis)
def _gelu(x):
    return jax.nn.gelu(x, approximate=True)
def _silu(x):
    return jax.nn.silu(x)
def _sigmoid(x):
    return jax.nn.sigmoid(x)
def _layernorm(x, axis=-1, eps=1e-5):
    m = jnp.mean(x, axis=axis, keepdims=True)
    v = jnp.var(x, axis=axis, keepdims=True)
    return (x - m) / jnp.sqrt(v + eps)
def _scatter_add(tgt, idx, src, axis=0):
    return tgt.at[idx].add(src)
def _segment_sum(src, seg, n):
    return jax.ops.segment_sum(src, seg, n)
class _Rng:
    def __init__(self, key):
        self._k = key
    def _next(self):
        self._k, sub = jax.random.split(self._k)
        return sub
    def normal(self, shape):
        return jax.random.normal(self._next(), shape, dtype=jnp.bfloat16)
    def randint(self, lo, hi, shape):
        return jax.random.randint(self._next(), shape, lo, hi, dtype=jnp.int32)
    def uniform(self, shape, lo=0.0, hi=1.0):
        return jax.random.uniform(self._next(), shape, jnp.bfloat16, lo, hi)
    def permutation(self, n):
        return jax.random.permutation(self._next(), n)


kernel_name = 'sequential_preLN__softmax_full_mha__dense_activation_squared_relu__prompt'

def setup_inputs():
    _rng = _Rng(jax.random.key(int.from_bytes(__import__("os").urandom(4), "little")))
    _w = (lambda a: (lambda t: t.astype(jnp.bfloat16) if jnp.issubdtype(t.dtype, jnp.floating) else t)(jnp.asarray(a)))
    def _A_setup():
        B, S, D = 1, 2048, 640
        return {
            "x": _w((lambda *s: _rng.normal(s) * 0.05)(B, S, D)),
            "wqkv": _w((lambda *s: _rng.normal(s) * 0.05)(D, 3 * D)),
            "wo": _w((lambda *s: _rng.normal(s) * 0.05)(D, D)),
        }
    _A_in = _A_setup()

    def _B_setup():
        B, S, D, F = 1, 2048, 640, 1536
        return {
            "x": _w((lambda *s: _rng.normal(s) * 0.05)(B, S, D)),
            "w1": _w((lambda *s: _rng.normal(s) * 0.05)(D, F)),
            "b1": _w((lambda *s: _rng.normal(s) * 0.05)(F)),
            "w2": _w((lambda *s: _rng.normal(s) * 0.05)(F, D)),
            "b2": _w((lambda *s: _rng.normal(s) * 0.05)(D)),
        }
    _B_in = _B_setup()

    return {
        "A_x": _A_in["x"],
        "A_wqkv": _A_in["wqkv"],
        "A_wo": _A_in["wo"],
        "B_x": _B_in["x"],
        "B_w1": _B_in["w1"],
        "B_b1": _B_in["b1"],
        "B_w2": _B_in["w2"],
        "B_b2": _B_in["b2"],
    }

def reference(A_x, A_wqkv, A_wo, B_x, B_w1, B_b1, B_w2, B_b2):
    def _A_ref(x, wqkv, wo):
        B, S, D = x.shape
        H = 32; Dh = D // H
        qkv = (lambda x, *d: x.transpose(*d))((x @ wqkv).reshape(B, S, 3, H, Dh), 2, 0, 3, 1, 4)
        q, k, v = qkv[0], qkv[1], qkv[2]
        scale = Dh ** -0.5
        scores = jnp.einsum("bhqd,bhkd->bhqk", q, k) * scale
        p = _softmax(scores, axis=-1)
        o = jnp.einsum("bhqk,bhkd->bhqd", p, v)
        return (lambda x, *d: x.transpose(*d))(o, 0, 2, 1, 3).reshape(B, S, D) @ wo

    def _B_ref(x, w1, b1, w2, b2):
        h = jnp.einsum("bsd,df->bsf", x, w1) + b1
        zero = jnp.zeros_like(h)
        r = jnp.where(h > zero, h, zero)
        h = r * r
        out = jnp.einsum("bsf,fd->bsd", h, w2) + b2
        return out

    x = A_x
    h = x + _A_ref(_layernorm(x, axis=-1), A_wqkv, A_wo)
    h2 = h + _B_ref(_layernorm(h, axis=-1), B_w1, B_b1, B_w2, B_b2)
    return h2
```

```python
import functools
import math

import jax
import jax.numpy as jnp
from jax import lax
import jax.experimental.pallas as pl
import jax.experimental.pallas.tpu as pltpu

F32, BF16 = jnp.float32, jnp.bfloat16

H = 32
DH = 20
WIN = 24
QT = 512
GK = 128
NV = 16
LAG = 2
NSLOT = 4
EPS = 1e-5
L_MIN, L_MAX = 2.0 ** -30, 2.0 ** 60

CFG = dict(MA=256, MC=256, stage="bf16", kpos=0.3, nk=1, dok=1, dof=1, fb=1, dmaj=1, ahead=1, xlu=1, only=-1, kskip=32, doc=1, npre=1)


def _layernorm(x):
    mean = jnp.mean(x, axis=-1, keepdims=True)
    xc = x - mean
    var = jnp.mean(xc * xc, axis=-1, keepdims=True)
    return xc * lax.rsqrt(var + EPS)


def _win_start(h):
    return DH * h - (DH * h) % 8


def _block_kernel(x_hbm, wqkv_hbm, wo_hbm, w1_hbm, b1_ref, w2_hbm, b2_ref, out_hbm, qrows_hbm,
                  x_v, wk_v, wqv_v, wqvt_v, wo_v, w1_v, w2_v, out_v,
                  kw, kv0, kv1, qw, qrows, qb, ow, acc_v, lrange, h_v, hn_v,
                  zero_s, sem_x, sem_w, sem_o, sem_q, sem_r, *p_slots, cfg):
    S, D = x_v.shape
    MA, MC = cfg["MA"], cfg["MC"]
    NQ, NG = S // QT, S // GK
    NM = GK - NV
    stage = cfg["stage"]

    def x_copy(i):
        return pltpu.make_async_copy(x_hbm.at[0, pl.ds(i * MA, MA), :], x_v.at[pl.ds(i * MA, MA), :], sem_x.at[i])

    w_copies = [
        pltpu.make_async_copy(wqkv_hbm.at[:, pl.ds(D, D)], wk_v, sem_w.at[0]),
        pltpu.make_async_copy(wqkv_hbm.at[:, pl.ds(0, D)], wqv_v.at[0], sem_w.at[1]),
        pltpu.make_async_copy(wqkv_hbm.at[:, pl.ds(2 * D, D)], wqv_v.at[1], sem_w.at[2]),
        pltpu.make_async_copy(wo_hbm, wo_v, sem_w.at[3]),
        pltpu.make_async_copy(w1_hbm, w1_v, sem_w.at[4]),
        pltpu.make_async_copy(w2_hbm, w2_v, sem_w.at[5]),
    ]
    x_copy(0).start()
    for c in w_copies[:3]:
        c.start()
    for i in range(1, S // MA):
        x_copy(i).start()
    for c in w_copies[3:]:
        c.start()

    for i in range(4 + NG):
        zero_s[i] = 0

    w_copies[1].wait()
    wqvt_v[pl.ds(0, D), :] = wqv_v[0].T
    w_copies[2].wait()
    wqvt_v[pl.ds(D, D), :] = wqv_v[1].T
    w_copies[0].wait()

    q_scale = DH ** -0.5 * math.log2(math.e)
    sub = lax.broadcasted_iota(jnp.int32, (8, MA), 0)

    NA = NV // 8
    NKB = NG * NA * DH
    NT = QT // 128
    n_items = 2 * NQ

    kvs = (kv0, kv1)
    SOFF = NKB + H // 2 * NG * 3

    def v_tile(h, odd, g):
        return kvs[1 - odd][pl.ds(NKB + (h // 2 * NG + g) * 3, 3)].reshape(WIN, GK)

    def window(src, b, odd, fill):
        mid = src[b + 16:b + 24]
        if odd:
            return jnp.concatenate([jnp.where(sub >= 4, mid, fill), src[b + 24:b + 40]], axis=0)
        return jnp.concatenate([src[b:b + 16], jnp.where(sub < 4, mid, fill)], axis=0)

    def rows_copy(i):
        n = MA // 128 * 2 * DH
        rows = pl.ds(pl.multiple_of(i * n, 8), n)
        return pltpu.make_async_copy(qrows.at[:, rows, :], qrows_hbm.at[:, rows, :], sem_r.at[i])

    NQB = S // 128 * 2 * DH

    def qkv_block(i, carry):
        x_copy(i).wait()
        r0 = pl.multiple_of(i * MA, MA)
        xn = _layernorm(x_v[pl.ds(r0, MA), :].astype(F32)).astype(BF16)
        k = jnp.dot(xn, wk_v[...], preferred_element_type=F32).astype(BF16)
        for h in range(H):
            kwin = k[:, _win_start(h):_win_start(h) + WIN]
            kw[h, pl.ds(r0, MA), :] = kwin
            for c in range(MA // GK):
                kvs[h % 2][pl.ds(SOFF + (h // 2 * NG + i * (MA // GK) + c) * NA, NA), :, pl.ds(0, WIN)] = (
                    kwin[c * GK + NM:(c + 1) * GK].astype(F32).reshape(NA, 8, WIN))
        qv = lax.dot_general(wqvt_v[...], xn, (((1,), (1,)), ((), ())), preferred_element_type=F32)
        q = (qv[:D] * q_scale).astype(BF16).astype(F32)
        v = qv[D:].astype(BF16).astype(F32)
        for p in range(H // 2):
            b = 2 * DH * p
            for odd in range(2):
                qwin, vwin = window(q, b, odd, 0.0), window(v, b, odd, 1.0)
                for c in range(MA // GK):
                    kvs[1 - odd][pl.ds(NKB + (p * NG + i * (MA // GK) + c) * 3, 3)] = vwin[:, c * GK:(c + 1) * GK].reshape(3, 8, GK)
                qw[2 * p + odd, :, pl.ds(r0, MA)] = qwin
            for c in range(MA // 128):
                qrows[p, pl.ds(pl.multiple_of((i * (MA // 128) + c) * 2 * DH, 8), 2 * DH), :] = q[b:b + 2 * DH, c * 128:(c + 1) * 128]
        for c in range(MA // 128):
            for p in range(cfg["npre"]):
                for r in range(2 * DH):
                    row = q[2 * DH * p + r:2 * DH * p + r + 1, c * 128:(c + 1) * 128]
                    qb[p * NQB + (i * (MA // 128) + c) * 2 * DH + r] = jnp.broadcast_to(row, (8, 128))
        rows_copy(i).start()
        return carry

    lax.fori_loop(0, S // MA, qkv_block, 0)


    def load_kb(p, odd, es, zl):
        todo = []
        for e in es:
            if cfg["dmaj"]:
                gd, a = divmod(e, NA)
                g, d = divmod(gd, DH)
                todo.append((g * NA + a, d))
            else:
                todo.append(divmod(e, DH))
        return todo, {ga: kvs[odd][zl + SOFF + p * NG * NA + ga] for ga in sorted({ga for ga, _ in todo})}

    def build_kb(odd, work, z):
        todo, src = work
        for ga, d in todo:
            c = 4 * odd + d
            kvs[odd][z + ga * DH + d] = jnp.broadcast_to(src[ga][:, c:c + 1], (8, 128)) if cfg['xlu'] else src[ga]

    NQB = S // 128 * 2 * DH

    def qb_copies(p):
        dst = qb.at[pl.ds((p % 2) * NQB, NQB)]
        return [pltpu.make_async_copy(qrows_hbm.at[p], dst.at[:, r, :], sem_q.at[r]) for r in range(8)]

    def finish(slot, odd, j, acc):
        l = jnp.broadcast_to(acc[0:1] if odd else acc[WIN - 1:WIN], (8, QT))
        lrange[0] = jnp.minimum(lrange[0], jnp.where(l >= L_MIN, l, 0.0))
        lrange[1] = jnp.maximum(lrange[1], l)
        inv = 1.0 / l
        ow[slot, :, pl.ds(j * QT, QT)] = acc * jnp.concatenate([inv] * (WIN // 8), axis=0)

    def pv(h, odd, g, slot, z):
        p = p_slots[slot][z, pl.ds(0, GK), :]
        return jnp.dot(v_tile(h, odd, g), p, preferred_element_type=F32)

    build_kb(0, load_kb(0, 0, range(NKB), 0), 0)
    for n in range(-LAG, 0):
        p_slots[n % NSLOT][0] = jnp.zeros(p_slots[0].shape[1:], p_slots[0].dtype)
    acc_v[...] = jnp.ones(acc_v.shape, F32)
    lrange[0] = jnp.ones((8, QT), F32)
    lrange[1] = jnp.ones((8, QT), F32)

    n_gran = n_items * NG
    period = NM + WIN
    events = [((k + 0.5) * 16 / period, "s", k) for k in range(NM // 16)]
    events += [((k + 0.5) / (QT // 128) + 1e-3, "v", k) for k in range(QT // 128)]
    events += [((NM + (k + 0.5) * WIN / 3) / period, "a", k) for k in range(3)]
    nk = cfg["nk"]
    events += [(cfg["kpos"] + k / nk, "k", k) for k in range(nk)]
    events.sort(key=lambda e: e[0])

    def pair_body(t, carry):
        @pl.when(t >= cfg["npre"])
        def _():
            for c in qb_copies(t):
                c.wait()

        @pl.when(t == cfg["npre"] - 1)
        def _():
            for i in range(S // MA):
                rows_copy(i).wait()

        @pl.when((t + 1 < H // 2) & (t + 1 >= cfg["npre"]))
        def _():
            for c in qb_copies(t + 1):
                c.start()

        za, zb, zc = zero_s[0], zero_s[1], zero_s[2]
        qb0 = (t % 2) * NQB
        acc = acc_v[...]
        kb_work = []
        for n in range(n_gran):
            u, g = divmod(n, NG)
            odd, j = divmod(u, NQ)
            h = 2 * t + odd
            s = jnp.dot(kw[h, pl.ds(g * GK, NM), :], qw[h, :, pl.ds(j * QT, QT)], preferred_element_type=F32)
            up, gp = divmod(n - LAG, NG)
            oddp, jp = divmod(up % n_items, NQ)
            hp = 2 * t + oddp if up >= 0 else jnp.maximum(2 * t - 1, 1)
            r = pv(hp, oddp, gp, (n - LAG) % NSLOT, zc)
            acc = r if gp == 0 else acc + r
            if gp == NG - 1 and cfg['dof']:
                finish(hp if up >= 0 else jnp.where(t == 0, H, hp), oddp, jp, acc)
            part = (j * NG + g) % (NQ * NG)
            hk = jnp.minimum(t + 1, H // 2 - 1) if odd else t
            ps = p_slots[n % NSLOT]
            for _, kind, k in events:
                if kind == "s":
                    ps[za, pl.ds(16 * k, 16), :] = jnp.exp2(s[16 * k:16 * k + 16]).astype(ps.dtype)
                elif kind == "k" and (not cfg["dok"] or cfg["only"] == 1 - odd):
                    pass
                elif kind == "k":
                    ahead = cfg["ahead"]
                    part -= cfg["kskip"] * odd
                    steps = NQ * NG - ahead - cfg["kskip"] * odd
                    if 0 <= part < steps:
                        kb_work.append(load_kb(hk, 1 - odd, range(part * NKB // steps, (part + 1) * NKB // steps), zc))
                    if part >= ahead:
                        build_kb(1 - odd, kb_work.pop(0), zb)
                elif kind == "a":
                    ps[za, pl.ds(GK + 8 * k, 8), :] = acc[8 * k:8 * k + 8].astype(ps.dtype)
                else:
                    sv = [None] * (NV // 8)
                    for d in range(DH):
                        qd = qb[qb0 + (j * NT + k) * 2 * DH + odd * DH + d]
                        for a in range(NA):
                            term = kvs[odd][zc + (g * NA + a) * DH + d] * qd
                            sv[a] = term if d == 0 else sv[a] + term
                    ps[zb, pl.ds(NM, NV), pl.ds(128 * k, 128)] = jnp.exp2(jnp.concatenate(sv, axis=0)).astype(ps.dtype)
        acc_v[...] = acc
        return carry

    lax.fori_loop(0, H // 2, pair_body, 0)
    acc = acc_v[...]
    for n in range(-LAG, 0):
        acc = acc + pv(H - 1, 1, NG + n, n % NSLOT, 0)
    finish(H - 1, 1, NQ - 1, acc)

    unsafe = jnp.logical_or(jnp.min(lrange[0]) < L_MIN, jnp.logical_not(jnp.max(lrange[1]) <= L_MAX))

    @pl.when(unsafe)
    def _():
        def item(i, carry):
            p, c = i // (S // 128), i % (S // 128)
            c0 = pl.multiple_of(c * 128, 128)
            for odd in range(2):
                h = 2 * p + odd
                vt = jnp.concatenate([v_tile(h, odd, g) for g in range(NG)], axis=1)
                s = jnp.dot(kw[h], qw[h, :, pl.ds(c0, 128)], preferred_element_type=F32)
                e = jnp.exp2(s - jnp.max(s, axis=0, keepdims=True)).astype(BF16)
                o = jnp.dot(vt, e, preferred_element_type=F32)
                l = o[0:1] if odd else o[WIN - 1:WIN]
                ow[h, :, pl.ds(c0, 128)] = o / l
            return carry

        if cfg["fb"]:
            lax.fori_loop(0, H // 2 * (S // 128), item, 0)

    for c in w_copies[3:]:
        c.wait()
    b1 = b1_ref[...].astype(F32).reshape(1, -1)
    b2 = b2_ref[...].astype(F32).reshape(1, -1)
    subc = lax.broadcasted_iota(jnp.int32, (8, MC), 0)

    def attn_out(i, slot):
        r0 = pl.multiple_of(i * MC, MC)
        rows = []
        for p in range(H // 2):
            even, oddw = [ow[2 * p + odd, :, pl.ds(r0, MC)] for odd in range(2)]
            rows += [even[:16], jnp.where(subc < 4, even[16:], oddw[:8]), oddw[8:]]
        o = jnp.concatenate(rows, axis=0).T.astype(BF16)
        hres = x_v[pl.ds(r0, MC), :].astype(F32) + jnp.dot(o, wo_v[...], preferred_element_type=F32)
        h_v[slot] = hres
        hn_v[slot] = _layernorm(hres).astype(BF16)

    def out_copy(i):
        r0 = pl.multiple_of(i * MC, MC)
        return pltpu.make_async_copy(out_v.at[pl.ds(r0, MC), :], out_hbm.at[0, pl.ds(r0, MC), :], sem_o.at[i])

    def ffn(i, slot):
        r0 = pl.multiple_of(i * MC, MC)
        a = jnp.dot(hn_v[slot], w1_v[...], preferred_element_type=F32) + b1
        a = jnp.where(a > 0.0, a, 0.0)
        y = jnp.dot((a * a).astype(BF16), w2_v[...], preferred_element_type=F32)
        out_v[pl.ds(r0, MC), :] = (h_v[slot] + (y + b2)).astype(out_v.dtype)

    nc = S // MC
    attn_out(0, 0)

    def ffn_block(i, carry):
        ffn(i, i % 2)
        attn_out(i + 1, (i + 1) % 2)
        out_copy(i).start()
        return carry

    if not cfg['doc']:
        out_copy(0).start()
        out_copy(0).wait()
        return
    lax.fori_loop(0, nc - 1, ffn_block, 0)
    ffn(nc - 1, (nc - 1) % 2)
    out_copy(nc - 1).start()
    for i in range(nc):
        out_copy(i).wait()


def _call(A_x, A_wqkv, A_wo, B_w1, B_b1, B_w2, B_b2, cfg, **kwargs):
    _, S, D = A_x.shape
    F = B_w1.shape[1]
    MA, MC = cfg["MA"], cfg["MC"]
    assert D == H * DH and S % QT == 0 and S % MA == 0 and S % MC == 0
    p_dtype = F32 if cfg["stage"] == "f32" else BF16
    any_spec = pl.BlockSpec(memory_space=pl.ANY)
    vmem_spec = pl.BlockSpec(memory_space=pltpu.VMEM)
    n_vgroups = S // GK * NV // 8
    scratch = [
        pltpu.VMEM((S, D), BF16),
        pltpu.VMEM((D, D), BF16),
        pltpu.VMEM((2, D, D), BF16),
        pltpu.VMEM((2 * D, D), BF16),
        pltpu.VMEM((D, D), BF16),
        pltpu.VMEM((D, F), BF16),
        pltpu.VMEM((F, D), BF16),
        pltpu.VMEM((S, D), A_x.dtype),
        pltpu.VMEM((H, S, WIN), BF16),
        pltpu.VMEM((n_vgroups * DH + H // 2 * (S // GK * 3 + n_vgroups), 8, 128), F32),
        pltpu.VMEM((n_vgroups * DH + H // 2 * (S // GK * 3 + n_vgroups), 8, 128), F32),
        pltpu.VMEM((H, WIN, S), F32),
        pltpu.VMEM((H // 2, S // 128 * 2 * DH, 128), F32),
        pltpu.VMEM((2 * S // 128 * 2 * DH, 8, 128), F32),
        pltpu.VMEM((H + 1, WIN, S), F32),
        pltpu.VMEM((WIN, QT), F32),
        pltpu.VMEM((2, 8, QT), F32),
        pltpu.VMEM((2, MC, D), F32),
        pltpu.VMEM((2, MC, D), BF16),
        pltpu.SMEM((4 + S // GK,), jnp.int32),
        pltpu.SemaphoreType.DMA((S // MA,)),
        pltpu.SemaphoreType.DMA((6,)),
        pltpu.SemaphoreType.DMA((S // MC,)),
        pltpu.SemaphoreType.DMA((8,)),
        pltpu.SemaphoreType.DMA((S // MA,)),
    ] + [pltpu.VMEM((2, GK + 32, QT), p_dtype)] * NSLOT
    return pl.pallas_call(
        functools.partial(_block_kernel, cfg=cfg),
        out_shape=(jax.ShapeDtypeStruct(A_x.shape, A_x.dtype),
                   jax.ShapeDtypeStruct((H // 2, S // 128 * 2 * DH, 128), F32)),
        in_specs=[any_spec, any_spec, any_spec, any_spec, vmem_spec, any_spec, vmem_spec],
        out_specs=(any_spec, any_spec),
        scratch_shapes=scratch,
        compiler_params=pltpu.CompilerParams(vmem_limit_bytes=110 * 2 ** 20),
        **kwargs,
    )(A_x, A_wqkv, A_wo, B_w1, B_b1, B_w2, B_b2)[0]


@jax.jit
def pallas_sequential_preLN__softmax_full_mha__dense_activation_squared_relu__prompt_kernel(
    A_x: jax.Array,
    A_wqkv: jax.Array,
    A_wo: jax.Array,
    B_x: jax.Array,
    B_w1: jax.Array,
    B_b1: jax.Array,
    B_w2: jax.Array,
    B_b2: jax.Array,
):
    del B_x
    return _call(A_x, A_wqkv, A_wo, B_w1, B_b1, B_w2, B_b2, CFG)
```

```python
import math

import jax
import jax.numpy as jnp
from jax import lax
import jax.experimental.pallas as pl
import jax.experimental.pallas.tpu as pltpu

F32, BF16 = jnp.float32, jnp.bfloat16

H = 32
DH = 20
WIN = 24
QT = 512
GK = 128
NV = 16
NA = NV // 8
NM = GK - NV
LAG = 2
NSLOT = 4
ROWS = 256
EPS = 1e-5
SUM_MIN, SUM_MAX = 2.0 ** -30, 2.0 ** 60

NN = (((1,), (0,)), ((), ()))
NT = (((1,), (1,)), ((), ()))


def _dot(a, b, dims=NN):
    return lax.dot_general(a.astype(BF16), b.astype(BF16), dims, preferred_element_type=F32)


def _layernorm(x):
    mean = jnp.mean(x, axis=-1, keepdims=True)
    xc = x - mean
    var = jnp.mean(xc * xc, axis=-1, keepdims=True)
    return xc * lax.rsqrt(var + EPS)


def _quadrants(a):
    r, c = a.shape[0] // 2, a.shape[1] // 2
    return a[:r, :c], a[:r, c:], a[r:, :c], a[r:, c:]


def _store_weight_sums(w_ref, sums_ref, part=0, parts=1):
    _, kh, nh = sums_ref.shape
    n = kh // parts
    r0 = pl.multiple_of(part * n, n) if parts > 1 else 0
    b11, b12, b21, b22 = [w_ref[pl.ds(r * kh + r0, n), pl.ds(c * nh, nh)].astype(F32)
                          for r in range(2) for c in range(2)]
    for i, s in enumerate((b11 + b22, b12 - b22, b21 - b11, b11 + b12, b21 + b22)):
        sums_ref[i, pl.ds(r0, n), :] = s.astype(BF16)


def _dense(a, w_ref, sums_ref):
    _, kh, nh = sums_ref.shape
    a11, a12, a21, a22 = _quadrants(a[:, :2 * kh])
    m1 = _dot(a11 + a22, sums_ref[0])
    m2 = _dot(a21 + a22, w_ref[pl.ds(0, kh), pl.ds(0, nh)])
    m4 = _dot(a22, sums_ref[2])
    c21, c11, c22 = m2 + m4, m1 + m4, m1 - m2
    m3 = _dot(a11, sums_ref[1])
    m5 = _dot(a11 + a12, w_ref[pl.ds(kh, kh), pl.ds(nh, nh)])
    c12 = m3 + m5
    c22 = c22 + m3 + _dot(a21 - a11, sums_ref[3])
    c11 = c11 - m5 + _dot(a12 - a22, sums_ref[4])
    out = jnp.concatenate([jnp.concatenate([c11, c12], axis=1), jnp.concatenate([c21, c22], axis=1)], axis=0)
    if 2 * nh < w_ref.shape[1]:
        rest = _dot(a[:, :2 * kh], w_ref[pl.ds(0, 2 * kh), pl.ds(2 * nh, w_ref.shape[1] - 2 * nh)])
        out = jnp.concatenate([out, rest], axis=1)
    if 2 * kh < w_ref.shape[0]:
        out = out + _dot(a[:, 2 * kh:], w_ref[pl.ds(2 * kh, w_ref.shape[0] - 2 * kh), :])
    return out


def _block_kernel(x_hbm, wqkv_hbm, wo_hbm, w1_hbm, b1_hbm, w2_hbm, b2_hbm, out_hbm, qrows_hbm,
                  x_v, wk_v, wqv_v, wqvt_v, wo_v, w1_v, w2_v, out_v, wk_s, wo_s, w1_s, w2_s, xn_v, k_v,
                  kw, kv0, kv1, vw, qw, qrows, qb, ow, acc_v, h_v, hn_v,
                  zero_s, sem_x, sem_w, sem_o, sem_q, sem_r, *rest):
    *p_slots, b1_v, b2_v = rest
    S, D = x_v.shape
    NQ, NG, NB = S // QT, S // GK, S // ROWS
    STEPS = NQ * NG
    NQB = S // 128 * 2 * DH
    kvs = (kv0, kv1)
    NKB = NG * NA * DH
    KSRC = NKB + H // 2 * NG * 3
    SPARE = KSRC + H // 2 * NG * NA

    def block(i):
        return pl.ds(pl.multiple_of(i * ROWS, ROWS), ROWS)

    def x_copy(i):
        return pltpu.make_async_copy(x_hbm.at[0, block(i), :], x_v.at[block(i), :], sem_x.at[i])

    def qrows_copy(i):
        n = ROWS // 128 * 2 * DH
        rows = pl.ds(pl.multiple_of(i * n, 8), n)
        return pltpu.make_async_copy(qrows.at[:, rows, :], qrows_hbm.at[:, rows, :], sem_r.at[i])

    def out_copy(i):
        return pltpu.make_async_copy(out_v.at[block(i), :], out_hbm.at[0, block(i), :], sem_o.at[i])

    wk_copy, wq_copy, wv_copy, *late_copies = [
        pltpu.make_async_copy(src, dst, sem_w.at[i]) for i, (src, dst) in enumerate([
            (wqkv_hbm.at[:, pl.ds(D, D)], wk_v), (wqkv_hbm.at[:, pl.ds(0, D)], wqv_v.at[0]),
            (wqkv_hbm.at[:, pl.ds(2 * D, D)], wqv_v.at[1]),
            (wo_hbm, wo_v), (w1_hbm, w1_v), (w2_hbm, w2_v), (b1_hbm, b1_v), (b2_hbm, b2_v)])]
    x_copy(0).start()
    wk_copy.start()
    for i in range(zero_s.shape[0]):
        zero_s[i] = 0

    def normalize(i):
        xn_v[block(i), :] = _layernorm(x_v[block(i), :].astype(F32)).astype(BF16)

    def project_keys(i):
        k_v[block(i), :] = _dense(xn_v[block(i), :].astype(F32), wk_v, wk_s).astype(BF16)

    x_copy(0).wait()
    x_copy(1).start()
    normalize(0)
    wk_copy.wait()
    _store_weight_sums(wk_v, wk_s)
    for i in range(2, NB):
        x_copy(i).start()

    def key_block(i, carry):
        x_copy(i + 1).wait()

        @pl.when(i == min(2, NB - 2))
        def _():
            wq_copy.start()
            wv_copy.start()

        project_keys(i)
        normalize(i + 1)
        return carry

    lax.fori_loop(0, NB - 1, key_block, 0)
    wq_copy.wait()
    wv_copy.wait()
    for c in late_copies:
        c.start()
    project_keys(NB - 1)
    wqvt_v[pl.ds(0, D), :] = wqv_v[0].T
    wqvt_v[pl.ds(D, D), :] = wqv_v[1].T

    q_scale = DH ** -0.5 * math.log2(math.e)
    sub = lax.broadcasted_iota(jnp.int32, (8, ROWS), 0)

    def window(src, b, odd, fill):
        mid = src[b + 16:b + 24]
        if odd:
            return jnp.concatenate([jnp.where(sub >= 4, mid, fill), src[b + 24:b + 40]], axis=0)
        return jnp.concatenate([src[b:b + 16], jnp.where(sub < 4, mid, fill)], axis=0)

    def query_value_block(i, carry):
        k = k_v[block(i), :]
        first = [DH * h - DH * h % 8 for h in range(H)]
        for h in range(H):
            pairs = pl.ds(pl.multiple_of(i * (ROWS // 2), ROWS // 2), ROWS // 2)
            kw[h, pairs, :] = pltpu.bitcast(k, jnp.uint32)[:, first[h]:first[h] + WIN]
        for c in range(ROWS // GK):
            rows = k[c * GK + NM:(c + 1) * GK].astype(F32)
            group = (i * (ROWS // GK) + c) * NA
            for h in range(H):
                at = KSRC + h // 2 * NG * NA + group
                kvs[h % 2][pl.ds(at, NA), :, pl.ds(0, WIN)] = rows[:, first[h]:first[h] + WIN].reshape(NA, 8, WIN)
            for d in range(DH):
                for a in range(NA):
                    kv0[(group + a) * DH + d] = jnp.broadcast_to(rows[8 * a:8 * a + 8, d:d + 1], (8, 128))

        xn = xn_v[block(i), :]
        qv = jnp.concatenate([_dot(wqvt_v[pl.ds(r, 128), :], xn, NT) for r in range(0, 2 * D, 128)], axis=0)
        q = (qv[:D] * q_scale).astype(BF16).astype(F32)
        v = qv[D:].astype(BF16).astype(F32)
        for p in range(H // 2):
            for c in range(ROWS // 128):
                at = pl.multiple_of((i * (ROWS // 128) + c) * 2 * DH, 8)
                qrows[p, pl.ds(at, 2 * DH), :] = q[2 * DH * p:2 * DH * (p + 1), c * 128:(c + 1) * 128]
        qrows_copy(i).start()
        for c in range(ROWS // 128):
            for r in range(2 * DH):
                at = (i * (ROWS // 128) + c) * 2 * DH + r
                qb[at] = jnp.broadcast_to(q[r:r + 1, c * 128:(c + 1) * 128], (8, 128))
        for p in range(H // 2):
            for odd in range(2):
                qw[2 * p + odd, :, block(i)] = window(q, 2 * DH * p, odd, 0.0)
                vwin = window(v, 2 * DH * p, odd, 1.0)
                vw[2 * p + odd, :, block(i)] = vwin
                for c in range(ROWS // GK):
                    at = NKB + (p * NG + i * (ROWS // GK) + c) * 3
                    kvs[1 - odd][pl.ds(at, 3)] = vwin[:, c * GK:(c + 1) * GK].reshape(3, 8, GK)
        return carry

    lax.fori_loop(0, NB // 2, lambda i, c: query_value_block(2 * i + 1, query_value_block(2 * i, c)), 0)
    for c in late_copies:
        c.wait()

    def keys(h, r0, n):
        return pltpu.bitcast(kw[h, pl.ds(r0 // 2, n // 2), :], BF16)

    for n in range(-LAG, 0):
        p_slots[n % NSLOT][0] = jnp.zeros(p_slots[0].shape[1:], BF16)
    acc_v[...] = jnp.ones(acc_v.shape, F32)

    period = NM + WIN
    events = [((k + 0.5) * 16 / period, "s", k) for k in range(NM // 16)]
    events += [(1.08 * (k + 0.5) / (QT // 128) + 1e-3, "v", k) for k in range(QT // 128)]
    events += [(0.97, "a", 0), (0.6, "k", 0)]
    events.sort(key=lambda e: e[0])

    def pair_body(t, carry):
        t_next = jnp.minimum(t + 1, H // 2 - 1)
        dst = qb.at[pl.ds((t + 1) % 2 * NQB, NQB)]
        next_qb = [pltpu.make_async_copy(qrows_hbm.at[t_next], dst.at[:, r, :], sem_q.at[r]) for r in range(8)]
        za, zb, zc = zero_s[0], zero_s[1], zero_s[2]
        qb0 = t % 2 * NQB
        acc = acc_v[...]
        pending = []
        for c in next_qb:
            c.start()
        for n in range(2 * STEPS):
            odd, step = divmod(n, STEPS)
            j, g = divmod(step, NG)
            h = 2 * t + odd
            s = jnp.dot(keys(h, g * GK, NM), qw[h, :, pl.ds(j * QT, QT)], preferred_element_type=F32)

            oddp, stepp = divmod((n - LAG) % (2 * STEPS), STEPS)
            jp, gp = divmod(stepp, NG)
            hp = 2 * t + oddp if n >= LAG else jnp.maximum(2 * t - 1, 1)
            build = step - STEPS // 2 * odd
            p = p_slots[(n - LAG) % NSLOT][zc, pl.ds(0, GK), :]
            if oddp == odd and build >= 0:
                vt = kvs[1 - odd][pl.ds(NKB + (hp // 2 * NG + gp) * 3, 3)].reshape(WIN, GK)
            else:
                vt = vw[hp, :, pl.ds(gp * GK, GK)]
            r = jnp.dot(vt, p, preferred_element_type=F32)
            acc = r if gp == 0 else acc + r
            if gp == NG - 1:
                ow[hp if n >= LAG else jnp.where(t == 0, H, hp), :, pl.ds(jp * QT, QT)] = acc

            ps = p_slots[n % NSLOT]
            for _, kind, k in events:
                if kind == "s":
                    ps[za, pl.ds(16 * k, 16), :] = jnp.exp2(s[16 * k:16 * k + 16]).astype(BF16)
                elif kind == "a":
                    ps[za, pl.ds(GK + 16, 8), pl.ds(0, 128)] = acc[16:, :128].astype(BF16)
                elif kind == "v":
                    sv = [None] * NA
                    zk = zero_s[3 + j]
                    for d in range(DH):
                        qd = qb[qb0 + (j * (QT // 128) + k) * 2 * DH + odd * DH + d]
                        for a in range(NA):
                            term = kvs[odd][zk + (g * NA + a) * DH + d] * qd
                            sv[a] = term if d == 0 else sv[a] + term
                    ps[zb, pl.ds(NM, NV), pl.ds(128 * k, 128)] = jnp.exp2(jnp.concatenate(sv, axis=0)).astype(BF16)
                else:
                    span = STEPS - 1 - STEPS // 2 * odd
                    if 0 <= build < span:
                        todo = [(e // NA // DH * NA + e % NA, e // NA % DH)
                                for e in range(build * NKB // span, (build + 1) * NKB // span)]
                        base = zc + KSRC + (t_next if odd else t) * NG * NA
                        pending.append((todo, {ga: kvs[1 - odd][base + ga, :, pl.ds(0, WIN)]
                                               for ga in sorted({ga for ga, _ in todo})}))
                    if 1 <= build <= span:
                        todo, src = pending.pop(0)
                        for ga, d in todo:
                            c = 4 * (1 - odd) + d
                            kvs[1 - odd][zb + ga * DH + d] = jnp.broadcast_to(src[ga][:, c:c + 1], (8, 128))
            if n == STEPS - 1:
                kv1[zb + SPARE] = s[32:40, :128]
        acc_v[...] = acc
        for w, sums in ((wo_v, wo_s), (w1_v, w1_s), (w2_v, w2_s)):
            _store_weight_sums(w, sums, t, H // 2)
        for c in next_qb:
            c.wait()
        return carry

    for i in range(NB):
        qrows_copy(i).wait()
    lax.fori_loop(0, H // 2, pair_body, 0)
    acc = acc_v[...]
    for n in range(-LAG, 0):
        acc = acc + jnp.dot(vw[H - 1, :, pl.ds((NG + n) * GK, GK)], p_slots[n % NSLOT][0, pl.ds(0, GK), :],
                            preferred_element_type=F32)
    ow[H - 1, :, pl.ds((NQ - 1) * QT, QT)] = acc

    def attention_out(i, slot):
        rows = []
        for p in range(H // 2):
            even, odd = ow[2 * p, :, block(i)], ow[2 * p + 1, :, block(i)]
            even = even * jnp.broadcast_to(1.0 / even[WIN - 1:WIN], (WIN, ROWS))
            odd = odd * jnp.broadcast_to(1.0 / odd[0:1], (WIN, ROWS))
            rows += [even[:16], jnp.where(sub < 4, even[16:], odd[:8]), odd[8:]]
        o = jnp.concatenate(rows, axis=0).T
        hres = x_v[block(i), :].astype(F32) + _dense(o, wo_v, wo_s)
        h_v[slot] = hres
        hn_v[slot] = _layernorm(hres)

    attention_out(0, 0)

    unsafe = jnp.zeros((8, S), F32)
    low = lax.broadcasted_iota(jnp.int32, (8, S), 0) < 4
    for p in range(H // 2):
        sums = jnp.where(low, ow[2 * p + 1, pl.ds(0, 8), :], ow[2 * p, pl.ds(WIN - 8, 8), :])
        unsafe = jnp.maximum(unsafe, jnp.where((sums >= SUM_MIN) & (sums <= SUM_MAX), 0.0, 1.0))

    @pl.when(jnp.max(unsafe) > 0.0)
    def _():
        def item(i, carry):
            h, cols = i // (S // 128), pl.ds(pl.multiple_of(i % (S // 128) * 128, 128), 128)
            s = jnp.dot(keys(h, 0, S), qw[h, :, cols], preferred_element_type=F32)
            e = jnp.exp2(s - jnp.max(s, axis=0, keepdims=True)).astype(BF16)
            ow[h, :, cols] = jnp.dot(vw[h], e, preferred_element_type=F32)
            return carry

        lax.fori_loop(0, H * (S // 128), item, 0)
        attention_out(0, 0)

    b1 = b1_v[...].astype(F32).reshape(1, -1)
    b2 = b2_v[...].astype(F32).reshape(1, -1)

    def ffn(i, slot, between=lambda: None):
        a = _dense(hn_v[slot], w1_v, w1_s) + b1
        a = jnp.where(a > 0.0, a, 0.0)
        between()
        y = _dense(a * a, w2_v, w2_s)
        out_v[block(i), :] = (h_v[slot] + (y + b2)).astype(out_v.dtype)

    def ffn_block(i, carry):
        ffn(i, i % 2, lambda: attention_out(i + 1, (i + 1) % 2))
        out_copy(i).start()
        return carry

    lax.fori_loop(0, NB - 1, ffn_block, 0)
    ffn(NB - 1, (NB - 1) % 2)
    out_copy(NB - 1).start()
    for i in range(NB):
        out_copy(i).wait()


def _block(x, wqkv, wo, w1, b1, w2, b2, **kwargs):
    _, S, D = x.shape
    F = w1.shape[1]
    assert x.shape[0] == 1 and D == H * DH and S % QT == 0
    dh, fh = D // 256 * 128, F // 256 * 128
    groups = S // GK * NA
    q_rows = S // 128 * 2 * DH
    kv_tiles = groups * DH + H // 2 * (S // GK * 3 + groups) + 8
    scratch = [
        pltpu.VMEM((S, D), BF16),
        pltpu.VMEM((D, D), BF16),
        pltpu.VMEM((2, D, D), BF16),
        pltpu.VMEM((2 * D, D), BF16),
        pltpu.VMEM((D, D), BF16),
        pltpu.VMEM((D, F), BF16),
        pltpu.VMEM((F, D), BF16),
        pltpu.VMEM((S, D), x.dtype),
        pltpu.VMEM((5, dh, dh), BF16),
        pltpu.VMEM((5, dh, dh), BF16),
        pltpu.VMEM((5, dh, fh), BF16),
        pltpu.VMEM((5, fh, dh), BF16),
        pltpu.VMEM((S, D), BF16),
        pltpu.VMEM((S, D), BF16),
        pltpu.VMEM((H, S // 2, WIN), jnp.uint32),
        pltpu.VMEM((kv_tiles, 8, 128), F32),
        pltpu.VMEM((kv_tiles, 8, 128), F32),
        pltpu.VMEM((H, WIN, S), F32),
        pltpu.VMEM((H, WIN, S), F32),
        pltpu.VMEM((H // 2, q_rows, 128), F32),
        pltpu.VMEM((2 * q_rows, 8, 128), F32),
        pltpu.VMEM((H + 1, WIN, S), F32),
        pltpu.VMEM((WIN, QT), F32),
        pltpu.VMEM((2, ROWS, D), F32),
        pltpu.VMEM((2, ROWS, D), F32),
        pltpu.SMEM((3 + S // QT,), jnp.int32),
        pltpu.SemaphoreType.DMA((S // ROWS,)),
        pltpu.SemaphoreType.DMA((8,)),
        pltpu.SemaphoreType.DMA((S // ROWS,)),
        pltpu.SemaphoreType.DMA((8,)),
        pltpu.SemaphoreType.DMA((S // ROWS,)),
    ] + [pltpu.VMEM((2, GK + 32, QT), BF16)] * NSLOT + [pltpu.VMEM((F,), BF16), pltpu.VMEM((D,), BF16)]
    any_spec = pl.BlockSpec(memory_space=pl.ANY)
    out, _ = pl.pallas_call(
        _block_kernel,
        out_shape=(jax.ShapeDtypeStruct(x.shape, x.dtype),
                   jax.ShapeDtypeStruct((H // 2, q_rows, 128), F32)),
        in_specs=[any_spec] * 7,
        out_specs=(any_spec, any_spec),
        scratch_shapes=scratch,
        compiler_params=pltpu.CompilerParams(vmem_limit_bytes=120 * 2 ** 20),
        **kwargs,
    )(x, wqkv, wo, w1, b1, w2, b2)
    return out


@jax.jit
def pallas_sequential_preLN__softmax_full_mha__dense_activation_squared_relu__prompt_kernel(
    A_x: jax.Array,
    A_wqkv: jax.Array,
    A_wo: jax.Array,
    B_x: jax.Array,
    B_w1: jax.Array,
    B_b1: jax.Array,
    B_w2: jax.Array,
    B_b2: jax.Array,
):
    del B_x
    return _block(A_x, A_wqkv, A_wo, B_w1, B_b1, B_w2, B_b2)
```

```python
import math

import jax
import jax.numpy as jnp
from jax import lax
import jax.experimental.pallas as pl
import jax.experimental.pallas.tpu as pltpu

F32, BF16 = jnp.float32, jnp.bfloat16

H = 32
DH = 20
WIN = 24
QT = 512
GK = 128
NV = 16
NA = NV // 8
NM = GK - NV
LAG = 2
NSLOT = 4
ROWS = 256
STORE_ORDER = "s0 v0 s1 s2 s3 v1 s4 k0 s5 v2 s6 v3 a0"
EPS = 1e-5
SUM_MIN, SUM_MAX = 2.0 ** -30, 2.0 ** 60

NN = (((1,), (0,)), ((), ()))
NT = (((1,), (1,)), ((), ()))


def _dot(a, b, dims=NN):
    return lax.dot_general(a.astype(BF16), b.astype(BF16), dims, preferred_element_type=F32)


def _layernorm(x):
    mean = jnp.mean(x, axis=-1, keepdims=True)
    xc = x - mean
    var = jnp.mean(xc * xc, axis=-1, keepdims=True)
    return xc * lax.rsqrt(var + EPS)


def _quadrants(a):
    r, c = a.shape[0] // 2, a.shape[1] // 2
    return a[:r, :c], a[:r, c:], a[r:, :c], a[r:, c:]


def _store_weight_sums(w_ref, sums_ref, part=0, parts=1):
    _, kh, nh = sums_ref.shape
    n = kh // parts
    r0 = pl.multiple_of(part * n, n) if parts > 1 else 0
    b11, b12, b21, b22 = [w_ref[pl.ds(r * kh + r0, n), pl.ds(c * nh, nh)].astype(F32)
                          for r in range(2) for c in range(2)]
    for i, s in enumerate((b11 + b22, b12 - b22, b21 - b11, b11 + b12, b21 + b22)):
        sums_ref[i, pl.ds(r0, n), :] = s.astype(BF16)


def _dense(a, w_ref, sums_ref):
    _, kh, nh = sums_ref.shape
    a11, a12, a21, a22 = _quadrants(a[:, :2 * kh])
    m1 = _dot(a11 + a22, sums_ref[0])
    m2 = _dot(a21 + a22, w_ref[pl.ds(0, kh), pl.ds(0, nh)])
    m4 = _dot(a22, sums_ref[2])
    c21, c11, c22 = m2 + m4, m1 + m4, m1 - m2
    m3 = _dot(a11, sums_ref[1])
    m5 = _dot(a11 + a12, w_ref[pl.ds(kh, kh), pl.ds(nh, nh)])
    c12 = m3 + m5
    c22 = c22 + m3 + _dot(a21 - a11, sums_ref[3])
    c11 = c11 - m5 + _dot(a12 - a22, sums_ref[4])
    out = jnp.concatenate([jnp.concatenate([c11, c12], axis=1), jnp.concatenate([c21, c22], axis=1)], axis=0)
    if 2 * nh < w_ref.shape[1]:
        rest = _dot(a[:, :2 * kh], w_ref[pl.ds(0, 2 * kh), pl.ds(2 * nh, w_ref.shape[1] - 2 * nh)])
        out = jnp.concatenate([out, rest], axis=1)
    if 2 * kh < w_ref.shape[0]:
        out = out + _dot(a[:, 2 * kh:], w_ref[pl.ds(2 * kh, w_ref.shape[0] - 2 * kh), :])
    return out


def _block_kernel(x_hbm, wqkv_hbm, wo_hbm, w1_hbm, b1_hbm, w2_hbm, b2_hbm, out_hbm, qrows_hbm,
                  x_v, wk_v, wqv_v, wqvt_v, wo_v, w1_v, w2_v, out_v, wk_s, wo_s, w1_s, w2_s, xn_v, k_v,
                  kw, kv0, kv1, vw, qw, qrows, qb, ow, acc_v, h_v, hn_v,
                  zero_s, sem_x, sem_w, sem_o, sem_q, sem_r, *rest):
    *p_slots, b1_v, b2_v = rest
    S, D = x_v.shape
    NQ, NG, NB = S // QT, S // GK, S // ROWS
    STEPS = NQ * NG
    NQB = S // 128 * 2 * DH
    kvs = (kv0, kv1)
    NKB = NG * NA * DH
    KSRC = NKB + H // 2 * NG * 3
    SPARE = KSRC + H // 2 * NG * NA

    def block(i):
        return pl.ds(pl.multiple_of(i * ROWS, ROWS), ROWS)

    def x_copy(i):
        return pltpu.make_async_copy(x_hbm.at[0, block(i), :], x_v.at[block(i), :], sem_x.at[i])

    def qrows_copy(i):
        n = ROWS // 128 * 2 * DH
        rows = pl.ds(pl.multiple_of(i * n, 8), n)
        return pltpu.make_async_copy(qrows.at[:, rows, :], qrows_hbm.at[:, rows, :], sem_r.at[i])

    def out_copy(i):
        return pltpu.make_async_copy(out_v.at[block(i), :], out_hbm.at[0, block(i), :], sem_o.at[i])

    wk_copy, wq_copy, wv_copy, *late_copies = [
        pltpu.make_async_copy(src, dst, sem_w.at[i]) for i, (src, dst) in enumerate([
            (wqkv_hbm.at[:, pl.ds(D, D)], wk_v), (wqkv_hbm.at[:, pl.ds(0, D)], wqv_v.at[0]),
            (wqkv_hbm.at[:, pl.ds(2 * D, D)], wqv_v.at[1]),
            (wo_hbm, wo_v), (w1_hbm, w1_v), (w2_hbm, w2_v), (b1_hbm, b1_v), (b2_hbm, b2_v)])]
    x_copy(0).start()
    wk_copy.start()
    for i in range(zero_s.shape[0]):
        zero_s[i] = 0

    def normalize(i):
        xn_v[block(i), :] = _layernorm(x_v[block(i), :].astype(F32)).astype(BF16)

    def project_keys(i):
        k_v[block(i), :] = _dense(xn_v[block(i), :].astype(F32), wk_v, wk_s).astype(BF16)

    x_copy(0).wait()
    x_copy(1).start()
    normalize(0)
    wk_copy.wait()
    _store_weight_sums(wk_v, wk_s)
    for i in range(2, NB):
        x_copy(i).start()

    def key_block(i, carry):
        x_copy(i + 1).wait()

        @pl.when(i == min(2, NB - 2))
        def _():
            wq_copy.start()
            wv_copy.start()

        project_keys(i)
        normalize(i + 1)
        return carry

    lax.fori_loop(0, NB - 1, key_block, 0)
    wq_copy.wait()
    wv_copy.wait()
    for c in late_copies:
        c.start()
    project_keys(NB - 1)
    wqvt_v[pl.ds(0, D), :] = wqv_v[0].T
    wqvt_v[pl.ds(D, D), :] = wqv_v[1].T

    q_scale = DH ** -0.5 * math.log2(math.e)
    sub = lax.broadcasted_iota(jnp.int32, (8, ROWS), 0)

    def window(src, b, odd, fill):
        mid = src[b + 16:b + 24]
        if odd:
            return jnp.concatenate([jnp.where(sub >= 4, mid, fill), src[b + 24:b + 40]], axis=0)
        return jnp.concatenate([src[b:b + 16], jnp.where(sub < 4, mid, fill)], axis=0)

    def query_value_block(i, carry):
        k = k_v[block(i), :]
        first = [DH * h - DH * h % 8 for h in range(H)]
        for h in range(H):
            pairs = pl.ds(pl.multiple_of(i * (ROWS // 2), ROWS // 2), ROWS // 2)
            kw[h, pairs, :] = pltpu.bitcast(k, jnp.uint32)[:, first[h]:first[h] + WIN]
        for c in range(ROWS // GK):
            rows = k[c * GK + NM:(c + 1) * GK].astype(F32)
            group = (i * (ROWS // GK) + c) * NA
            for h in range(H):
                at = KSRC + h // 2 * NG * NA + group
                kvs[h % 2][pl.ds(at, NA), :, pl.ds(0, WIN)] = rows[:, first[h]:first[h] + WIN].reshape(NA, 8, WIN)
            for d in range(DH):
                for a in range(NA):
                    kv0[(group + a) * DH + d] = jnp.broadcast_to(rows[8 * a:8 * a + 8, d:d + 1], (8, 128))

        xn = xn_v[block(i), :]
        qv = jnp.concatenate([_dot(wqvt_v[pl.ds(r, 128), :], xn, NT) for r in range(0, 2 * D, 128)], axis=0)
        q = (qv[:D] * q_scale).astype(BF16).astype(F32)
        v = qv[D:].astype(BF16).astype(F32)
        for p in range(H // 2):
            for c in range(ROWS // 128):
                at = pl.multiple_of((i * (ROWS // 128) + c) * 2 * DH, 8)
                qrows[p, pl.ds(at, 2 * DH), :] = q[2 * DH * p:2 * DH * (p + 1), c * 128:(c + 1) * 128]
        qrows_copy(i).start()
        for c in range(ROWS // 128):
            for r in range(2 * DH):
                at = (i * (ROWS // 128) + c) * 2 * DH + r
                qb[at] = jnp.broadcast_to(q[r:r + 1, c * 128:(c + 1) * 128], (8, 128))
        for p in range(H // 2):
            for odd in range(2):
                qw[2 * p + odd, :, block(i)] = window(q, 2 * DH * p, odd, 0.0)
                vwin = window(v, 2 * DH * p, odd, 1.0)
                vw[2 * p + odd, :, block(i)] = vwin
                for c in range(ROWS // GK):
                    at = NKB + (p * NG + i * (ROWS // GK) + c) * 3
                    kvs[1 - odd][pl.ds(at, 3)] = vwin[:, c * GK:(c + 1) * GK].reshape(3, 8, GK)
        return carry

    lax.fori_loop(0, NB // 2, lambda i, c: query_value_block(2 * i + 1, query_value_block(2 * i, c)), 0)
    for c in late_copies:
        c.wait()

    def keys(h, r0, n):
        return pltpu.bitcast(kw[h, pl.ds(r0 // 2, n // 2), :], BF16)

    for n in range(-LAG, 0):
        p_slots[n % NSLOT][0] = jnp.zeros(p_slots[0].shape[1:], BF16)
    acc_v[...] = jnp.ones(acc_v.shape, F32)

    events = [(e[0], int(e[1])) for e in STORE_ORDER.split()]

    def pair_body(t, carry):
        t_next = jnp.minimum(t + 1, H // 2 - 1)
        dst = qb.at[pl.ds((t + 1) % 2 * NQB, NQB)]
        next_qb = [pltpu.make_async_copy(qrows_hbm.at[t_next], dst.at[:, r, :], sem_q.at[r]) for r in range(8)]
        za, zb, zc = zero_s[0], zero_s[1], zero_s[2]
        qb0 = t % 2 * NQB
        acc = acc_v[...]
        pending = []
        for c in next_qb:
            c.start()
        for n in range(2 * STEPS):
            odd, step = divmod(n, STEPS)
            j, g = divmod(step, NG)
            h = 2 * t + odd
            s = jnp.dot(keys(h, g * GK, NM), qw[h, :, pl.ds(j * QT, QT)], preferred_element_type=F32)

            oddp, stepp = divmod((n - LAG) % (2 * STEPS), STEPS)
            jp, gp = divmod(stepp, NG)
            hp = 2 * t + oddp if n >= LAG else jnp.maximum(2 * t - 1, 1)
            build = step - STEPS // 2 * odd
            p = p_slots[(n - LAG) % NSLOT][zc, pl.ds(0, GK), :]
            if oddp == odd and build >= 0:
                vt = kvs[1 - odd][pl.ds(NKB + (hp // 2 * NG + gp) * 3, 3)].reshape(WIN, GK)
            else:
                vt = vw[hp, :, pl.ds(gp * GK, GK)]
            r = jnp.dot(vt, p, preferred_element_type=F32)
            acc = r if gp == 0 else acc + r
            if gp == NG - 1:
                ow[hp if n >= LAG else jnp.where(t == 0, H, hp), :, pl.ds(jp * QT, QT)] = acc

            ps = p_slots[n % NSLOT]
            for kind, k in events:
                if kind == "s":
                    ps[za, pl.ds(16 * k, 16), :] = jnp.exp2(s[16 * k:16 * k + 16]).astype(BF16)
                elif kind == "a":
                    ps[za, pl.ds(GK + 16, 8), pl.ds(0, 128)] = acc[16:, :128].astype(BF16)
                elif kind == "v":
                    sv = [None] * NA
                    zk = zero_s[3 + j]
                    for d in (reversed(range(DH)) if g % 2 else range(DH)):
                        qd = qb[qb0 + (j * (QT // 128) + k) * 2 * DH + odd * DH + d]
                        for a in range(NA):
                            term = kvs[odd][zk + (g * NA + a) * DH + d] * qd
                            sv[a] = term if sv[a] is None else sv[a] + term
                    ps[zb, pl.ds(NM, NV), pl.ds(128 * k, 128)] = jnp.exp2(jnp.concatenate(sv, axis=0)).astype(BF16)
                else:
                    span = STEPS - 1 - STEPS // 2 * odd
                    if 0 <= build < span:
                        todo = [(e // NA // DH * NA + e % NA, e // NA % DH)
                                for e in range(build * NKB // span, (build + 1) * NKB // span)]
                        base = zc + KSRC + (t_next if odd else t) * NG * NA
                        pending.append((todo, {ga: kvs[1 - odd][base + ga, :, pl.ds(0, WIN)]
                                               for ga in sorted({ga for ga, _ in todo})}))
                    if 1 <= build <= span:
                        todo, src = pending.pop(0)
                        for ga, d in todo:
                            c = 4 * (1 - odd) + d
                            kvs[1 - odd][zb + ga * DH + d] = jnp.broadcast_to(src[ga][:, c:c + 1], (8, 128))
            if n == STEPS - 1:
                kv1[zb + SPARE] = s[8:16, :128]
        acc_v[...] = acc
        for w, sums in ((wo_v, wo_s), (w1_v, w1_s), (w2_v, w2_s)):
            _store_weight_sums(w, sums, t, H // 2)
        for c in next_qb:
            c.wait()
        return carry

    for i in range(NB):
        qrows_copy(i).wait()
    lax.fori_loop(0, H // 2, pair_body, 0)
    acc = acc_v[...]
    for n in range(-LAG, 0):
        acc = acc + jnp.dot(vw[H - 1, :, pl.ds((NG + n) * GK, GK)], p_slots[n % NSLOT][0, pl.ds(0, GK), :],
                            preferred_element_type=F32)
    ow[H - 1, :, pl.ds((NQ - 1) * QT, QT)] = acc

    def attention_out(i, slot):
        rows = []
        for p in range(H // 2):
            even, odd = ow[2 * p, :, block(i)], ow[2 * p + 1, :, block(i)]
            even = even * jnp.broadcast_to(1.0 / even[WIN - 1:WIN], (WIN, ROWS))
            odd = odd * jnp.broadcast_to(1.0 / odd[0:1], (WIN, ROWS))
            rows += [even[:16], jnp.where(sub < 4, even[16:], odd[:8]), odd[8:]]
        o = jnp.concatenate(rows, axis=0).T
        hres = x_v[block(i), :].astype(F32) + _dense(o, wo_v, wo_s)
        h_v[slot] = hres
        hn_v[slot] = _layernorm(hres)

    attention_out(0, 0)

    unsafe = jnp.zeros((8, S), F32)
    low = lax.broadcasted_iota(jnp.int32, (8, S), 0) < 4
    for p in range(H // 2):
        sums = jnp.where(low, ow[2 * p + 1, pl.ds(0, 8), :], ow[2 * p, pl.ds(WIN - 8, 8), :])
        unsafe = jnp.maximum(unsafe, jnp.where((sums >= SUM_MIN) & (sums <= SUM_MAX), 0.0, 1.0))

    @pl.when(jnp.max(unsafe) > 0.0)
    def _():
        def item(i, carry):
            h, cols = i // (S // 128), pl.ds(pl.multiple_of(i % (S // 128) * 128, 128), 128)
            s = jnp.dot(keys(h, 0, S), qw[h, :, cols], preferred_element_type=F32)
            e = jnp.exp2(s - jnp.max(s, axis=0, keepdims=True)).astype(BF16)
            ow[h, :, cols] = jnp.dot(vw[h], e, preferred_element_type=F32)
            return carry

        lax.fori_loop(0, H * (S // 128), item, 0)
        attention_out(0, 0)

    b1 = b1_v[...].astype(F32).reshape(1, -1)
    b2 = b2_v[...].astype(F32).reshape(1, -1)

    def ffn(i, slot, between=lambda: None):
        a = _dense(hn_v[slot], w1_v, w1_s) + b1
        a = jnp.where(a > 0.0, a, 0.0)
        between()
        y = _dense(a * a, w2_v, w2_s)
        out_v[block(i), :] = (h_v[slot] + (y + b2)).astype(out_v.dtype)

    def ffn_block(i, carry):
        ffn(i, i % 2, lambda: attention_out(i + 1, (i + 1) % 2))
        out_copy(i).start()
        return carry

    lax.fori_loop(0, NB - 1, ffn_block, 0)
    ffn(NB - 1, (NB - 1) % 2)
    out_copy(NB - 1).start()
    for i in range(NB):
        out_copy(i).wait()


def _block(x, wqkv, wo, w1, b1, w2, b2, **kwargs):
    _, S, D = x.shape
    F = w1.shape[1]
    assert x.shape[0] == 1 and D == H * DH and S % QT == 0
    dh, fh = D // 256 * 128, F // 256 * 128
    groups = S // GK * NA
    q_rows = S // 128 * 2 * DH
    kv_tiles = groups * DH + H // 2 * (S // GK * 3 + groups) + 8
    scratch = [
        pltpu.VMEM((S, D), BF16),
        pltpu.VMEM((D, D), BF16),
        pltpu.VMEM((2, D, D), BF16),
        pltpu.VMEM((2 * D, D), BF16),
        pltpu.VMEM((D, D), BF16),
        pltpu.VMEM((D, F), BF16),
        pltpu.VMEM((F, D), BF16),
        pltpu.VMEM((S, D), x.dtype),
        pltpu.VMEM((5, dh, dh), BF16),
        pltpu.VMEM((5, dh, dh), BF16),
        pltpu.VMEM((5, dh, fh), BF16),
        pltpu.VMEM((5, fh, dh), BF16),
        pltpu.VMEM((S, D), BF16),
        pltpu.VMEM((S, D), BF16),
        pltpu.VMEM((H, S // 2, WIN), jnp.uint32),
        pltpu.VMEM((kv_tiles, 8, 128), F32),
        pltpu.VMEM((kv_tiles, 8, 128), F32),
        pltpu.VMEM((H, WIN, S), F32),
        pltpu.VMEM((H, WIN, S), F32),
        pltpu.VMEM((H // 2, q_rows, 128), F32),
        pltpu.VMEM((2 * q_rows, 8, 128), F32),
        pltpu.VMEM((H + 1, WIN, S), F32),
        pltpu.VMEM((WIN, QT), F32),
        pltpu.VMEM((2, ROWS, D), F32),
        pltpu.VMEM((2, ROWS, D), F32),
        pltpu.SMEM((3 + S // QT,), jnp.int32),
        pltpu.SemaphoreType.DMA((S // ROWS,)),
        pltpu.SemaphoreType.DMA((8,)),
        pltpu.SemaphoreType.DMA((S // ROWS,)),
        pltpu.SemaphoreType.DMA((8,)),
        pltpu.SemaphoreType.DMA((S // ROWS,)),
    ] + [pltpu.VMEM((2, GK + 32, QT), BF16)] * NSLOT + [pltpu.VMEM((F,), BF16), pltpu.VMEM((D,), BF16)]
    any_spec = pl.BlockSpec(memory_space=pl.ANY)
    out, _ = pl.pallas_call(
        _block_kernel,
        out_shape=(jax.ShapeDtypeStruct(x.shape, x.dtype),
                   jax.ShapeDtypeStruct((H // 2, q_rows, 128), F32)),
        in_specs=[any_spec] * 7,
        out_specs=(any_spec, any_spec),
        scratch_shapes=scratch,
        compiler_params=pltpu.CompilerParams(vmem_limit_bytes=120 * 2 ** 20),
        **kwargs,
    )(x, wqkv, wo, w1, b1, w2, b2)
    return out


@jax.jit
def pallas_sequential_preLN__softmax_full_mha__dense_activation_squared_relu__prompt_kernel(
    A_x: jax.Array,
    A_wqkv: jax.Array,
    A_wo: jax.Array,
    B_x: jax.Array,
    B_w1: jax.Array,
    B_b1: jax.Array,
    B_w2: jax.Array,
    B_b2: jax.Array,
):
    del B_x
    return _block(A_x, A_wqkv, A_wo, B_w1, B_b1, B_w2, B_b2)
```
